```python
import os as _os
_os.environ.setdefault("JAX_PLATFORMS", "cpu")
import jax
import jax.numpy as jnp

def _softmax(x, axis=-1):
    return jax.nn.softmax(x, axis=axis)
def _gelu(x):
    return jax.nn.gelu(x, approximate=True)
def _silu(x):
    return jax.nn.silu(x)
def _sigmoid(x):
    return jax.nn.sigmoid(x)
def _layernorm(x, axis=-1, eps=1e-5):
    m = jnp.mean(x, axis=axis, keepdims=True)
    v = jnp.var(x, axis=axis, keepdims=True)
    return (x - m) / jnp.sqrt(v + eps)
def _scatter_add(tgt, idx, src, axis=0):
    return tgt.at[idx].add(src)
def _segment_sum(src, seg, n):
    return jax.ops.segment_sum(src, seg, n)
class _Rng:
    def __init__(self, key):
        self._k = key
    def _next(self):
        self._k, sub = jax.random.split(self._k)
        return sub
    def normal(self, shape):
        return jax.random.normal(self._next(), shape, dtype=jnp.bfloat16)
    def randint(self, lo, hi, shape):
        return jax.random.randint(self._next(), shape, lo, hi, dtype=jnp.int32)
    def uniform(self, shape, lo=0.0, hi=1.0):
        return jax.random.uniform(self._next(), shape, jnp.bfloat16, lo, hi)
    def permutation(self, n):
        return jax.random.permutation(self._next(), n)


kernel_name = 'sequential_preLN__softmax_full_mha__glu_gated_swiglu__prompt'

def setup_inputs():
    _rng = _Rng(jax.random.key(int.from_bytes(__import__("os").urandom(4), "little")))
    _w = (lambda a: (lambda t: t.astype(jnp.bfloat16) if jnp.issubdtype(t.dtype, jnp.floating) else t)(jnp.asarray(a)))
    def _A_setup():
        B, S, D = 1, 2048, 640
        return {
            "x": _w((lambda *s: _rng.normal(s) * 0.05)(B, S, D)),
            "wqkv": _w((lambda *s: _rng.normal(s) * 0.05)(D, 3 * D)),
            "wo": _w((lambda *s: _rng.normal(s) * 0.05)(D, D)),
        }
    _A_in = _A_setup()

    def _B_setup():
        B, S, D, F = 1, 2048, 640, 1728
        return {
            "x": _w((lambda *s: _rng.normal(s) * 0.05)(B, S, D)),
            "w1": _w((lambda *s: _rng.normal(s) * 0.05)(D, F) * (2.0 / D) ** 0.5),
            "w3": _w((lambda *s: _rng.normal(s) * 0.05)(D, F) * (2.0 / D) ** 0.5),
            "w2": _w((lambda *s: _rng.normal(s) * 0.05)(F, D) * (2.0 / F) ** 0.5),
        }
    _B_in = _B_setup()

    return {
        "A_x": _A_in["x"],
        "A_wqkv": _A_in["wqkv"],
        "A_wo": _A_in["wo"],
        "B_x": _B_in["x"],
        "B_w1": _B_in["w1"],
        "B_w3": _B_in["w3"],
        "B_w2": _B_in["w2"],
    }

def reference(A_x, A_wqkv, A_wo, B_x, B_w1, B_w3, B_w2):
    def _A_ref(x, wqkv, wo):
        B, S, D = x.shape
        H = 32; Dh = D // H
        qkv = (lambda x, *d: x.transpose(*d))((x @ wqkv).reshape(B, S, 3, H, Dh), 2, 0, 3, 1, 4)
        q, k, v = qkv[0], qkv[1], qkv[2]
        scale = Dh ** -0.5
        scores = jnp.einsum("bhqd,bhkd->bhqk", q, k) * scale
        p = _softmax(scores, axis=-1)
        o = jnp.einsum("bhqk,bhkd->bhqd", p, v)
        return (lambda x, *d: x.transpose(*d))(o, 0, 2, 1, 3).reshape(B, S, D) @ wo

    def _B_ref(x, w1, w3, w2):
        gate = jnp.einsum("bsd,df->bsf", x, w1)
        up = jnp.einsum("bsd,df->bsf", x, w3)
        h = _silu(gate) * up
        out = jnp.einsum("bsf,fd->bsd", h, w2)
        return out

    x = A_x
    h = x + _A_ref(_layernorm(x, axis=-1), A_wqkv, A_wo)
    h2 = h + _B_ref(_layernorm(h, axis=-1), B_w1, B_w3, B_w2)
    return h2
```

```python
import math
import jax
import jax.numpy as jnp
import jax.experimental.pallas as pl
import jax.experimental.pallas.tpu as pltpu

S, D, H, DH, F = 2048, 640, 32, 20, 1728
HPG = 6
NG = 6
GW = NG * 128
QB = 512
NQB = S // QB
RC = 256
KC = 128
NKC = S // KC
EPS = 1e-5
UN = 8
QSCALE = (DH ** -0.5) * math.log2(math.e)

NT = (((1,), (1,)), ((), ()))


def _ln(x):
    m = jnp.mean(x, axis=-1, keepdims=True)
    xc = x - m
    v = jnp.mean(xc * xc, axis=-1, keepdims=True)
    return xc * jax.lax.rsqrt(v + EPS)


def kernel(x_ref, wqkv_ref, wo_hbm, w1_hbm, w3_hbm, w2_hbm, o_ref,
           wg_ref, wvT_ref, k2_ref, q2_ref, vtp_ref, ot_ref, sa_ref, sb_ref, ma_ref, mb_ref,
           wo_ref, w1_ref, w3_ref, w2_ref, sems):
    step = pl.program_id(0)

    def late_copies():
        return [pltpu.make_async_copy(wo_hbm, wo_ref, sems.at[0]),
                pltpu.make_async_copy(w1_hbm, w1_ref, sems.at[1]),
                pltpu.make_async_copy(w3_hbm, w3_ref, sems.at[2]),
                pltpu.make_async_copy(w2_hbm, w2_ref, sems.at[3])]

    lane = jax.lax.broadcasted_iota(jnp.int32, (QB, 128), 1)

    def qweights(qbi, h):
        g = h // HPG
        j = h - g * HPG
        c0 = pl.multiple_of(g * 128, 128)
        lo = j * DH
        msk = (lane >= lo) & (lane < lo + DH)
        qq = q2_ref[pl.ds(pl.multiple_of(qbi * QB, QB), QB), pl.ds(c0, 128)]
        return jnp.where(msk, qq, jnp.zeros_like(qq)), c0

    def qk_chunk(qq, c0, sref, c, mx):
        kc = k2_ref[pl.ds(c * KC, KC), pl.ds(c0, 128)]
        s = jax.lax.dot_general(kc, qq, NT, preferred_element_type=jnp.float32)
        sref[pl.ds(c * KC, KC), :] = s
        sm = jnp.max(s.reshape(KC // 8, 8, QB), axis=0)
        return sm if mx is None else jnp.maximum(mx, sm)

    @pl.when(step == 0)
    def _phase1():
        for cp in late_copies():
            cp.start()
        for g in range(NG):
            wg_ref[:, g * 128:(g + 1) * 128] = wqkv_ref[:, g * 120:g * 120 + 128]
            wg_ref[:, GW + g * 128:GW + (g + 1) * 128] = wqkv_ref[:, D + g * 120:D + g * 120 + 128]
        wvT_ref[...] = wqkv_ref[:, 2 * D:3 * D].astype(jnp.float32).T.astype(jnp.bfloat16)

        def chunk(c, carry):
            r0 = pl.multiple_of(c * RC, RC)
            x = x_ref[pl.ds(r0, RC), :].astype(jnp.float32)
            xl = _ln(x).astype(jnp.bfloat16)
            qk = jnp.dot(xl, wg_ref[...], preferred_element_type=jnp.float32)
            q2_ref[pl.ds(r0, RC), :] = (qk[:, :GW] * QSCALE).astype(jnp.bfloat16)
            k2_ref[pl.ds(r0, RC), :] = qk[:, GW:].astype(jnp.bfloat16)
            vt = jax.lax.dot_general(wvT_ref[...], xl, NT, preferred_element_type=jnp.float32)
            row = jax.lax.broadcasted_iota(jnp.int32, (32, RC), 0)
            for h in range(H):
                a = (20 * h // 8) * 8
                off = 20 * h - a
                win = vt[a:a + 24, :]
                if off:
                    win = pltpu.roll(win, 24 - off, 0)
                win = jnp.concatenate([win, jnp.zeros((8, RC), jnp.float32)], axis=0)
                val = jnp.where(row < DH, win, jnp.where(row == DH, 1.0, 0.0))
                vtp_ref[h, :, pl.ds(r0, RC)] = val.astype(jnp.bfloat16)
            return carry
        jax.lax.fori_loop(0, S // RC, chunk, 0)

        qq, c0 = qweights(0, 0)
        mx = None
        for c in range(NKC):
            mx = qk_chunk(qq, c0, sa_ref, c, mx)
        ma_ref[...] = jnp.max(mx, axis=0, keepdims=True)

    @pl.when(step > 0)
    def _qblock():
        qb = step - 1
        q0 = pl.multiple_of(qb * QB, QB)

        def unit(h, qbn, hn, sc_ref, mc_ref, sn_ref, mn_ref):
            qq, c0 = qweights(qbn, hn)
            m = mc_ref[...]
            vt = vtp_ref[h]
            acc = jnp.zeros((32, QB), jnp.float32)
            mx = None
            for c in range(NKC):
                mx = qk_chunk(qq, c0, sn_ref, c, mx)
                sc = sc_ref[pl.ds(c * KC, KC), :]
                p = jnp.exp2(sc - m).astype(jnp.bfloat16)
                acc = acc + jnp.dot(vt[:, c * KC:(c + 1) * KC], p, preferred_element_type=jnp.float32)
            mn_ref[...] = jnp.max(mx, axis=0, keepdims=True)
            ot_ref[h, pl.ds(0, DH), :] = acc[:DH] / acc[DH:DH + 1]

        def pair(i, carry):
            h0 = UN * i
            last = i == H // UN - 1
            for u in range(UN):
                h = h0 + u
                bufs = (sa_ref, ma_ref, sb_ref, mb_ref) if u % 2 == 0 else (sb_ref, mb_ref, sa_ref, ma_ref)
                if u < UN - 1:
                    unit(h, qb, h + 1, *bufs)
                else:
                    qbn = jnp.where(last, jnp.minimum(qb + 1, NQB - 1), qb)
                    hn = jnp.where(last, 0, h + 1)
                    unit(h, qbn, hn, *bufs)
            return carry
        jax.lax.fori_loop(0, H // UN, pair, 0)

        @pl.when(step == 1)
        def _():
            for cp in late_copies():
                cp.wait()

        otf = jnp.concatenate([ot_ref[hh, 0:DH, :] for hh in range(H)], axis=0)
        attn = jnp.dot(otf.T.astype(jnp.bfloat16), wo_ref[...], preferred_element_type=jnp.float32)
        hres = x_ref[pl.ds(q0, QB), :].astype(jnp.float32) + attn
        l2 = _ln(hres).astype(jnp.bfloat16)
        gate = jax.lax.dot_general(l2, w1_ref[...], NT, preferred_element_type=jnp.float32)
        up = jax.lax.dot_general(l2, w3_ref[...], NT, preferred_element_type=jnp.float32)
        hf = (gate * jax.nn.sigmoid(gate) * up).astype(jnp.bfloat16)
        out = jnp.dot(hf, w2_ref[...], preferred_element_type=jnp.float32)
        o_ref[...] = (hres + out).astype(o_ref.dtype)


@jax.jit
def pallas_sequential_preLN__softmax_full_mha__glu_gated_swiglu__prompt_kernel(
    A_x: jax.Array,
    A_wqkv: jax.Array,
    A_wo: jax.Array,
    B_x: jax.Array,
    B_w1: jax.Array,
    B_w3: jax.Array,
    B_w2: jax.Array,
):
    x = A_x.reshape(S, D)
    full = lambda shp: pl.BlockSpec(shp, lambda i: (0,) * len(shp))
    anyspec = pl.BlockSpec(memory_space=pl.ANY)
    out = pl.pallas_call(
        kernel,
        grid=(1 + NQB,),
        in_specs=[full((S, D)), full((D, 3 * D)), anyspec, anyspec, anyspec, anyspec],
        out_specs=pl.BlockSpec((QB, D), lambda i: (jnp.maximum(i - 1, 0), 0)),
        out_shape=jax.ShapeDtypeStruct((S, D), jnp.bfloat16),
        scratch_shapes=[
            pltpu.VMEM((D, 2 * GW), jnp.bfloat16),
            pltpu.VMEM((D, D), jnp.bfloat16),
            pltpu.VMEM((S, GW), jnp.bfloat16),
            pltpu.VMEM((S, GW), jnp.bfloat16),
            pltpu.VMEM((H, 32, S), jnp.bfloat16),
            pltpu.VMEM((H, 24, QB), jnp.float32),
            pltpu.VMEM((S, QB), jnp.float32),
            pltpu.VMEM((S, QB), jnp.float32),
            pltpu.VMEM((1, QB), jnp.float32),
            pltpu.VMEM((1, QB), jnp.float32),
            pltpu.VMEM((D, D), jnp.bfloat16),
            pltpu.VMEM((F, D), jnp.bfloat16),
            pltpu.VMEM((F, D), jnp.bfloat16),
            pltpu.VMEM((F, D), jnp.bfloat16),
            pltpu.SemaphoreType.DMA((4,)),
        ],
        compiler_params=pltpu.CompilerParams(dimension_semantics=("arbitrary",),
                                             vmem_limit_bytes=100 * 1024 * 1024),
    )(x, A_wqkv, A_wo, B_w1.T, B_w3.T, B_w2)
    return out.reshape(1, S, D)
```

```python
import math

import jax
import jax.numpy as jnp
import jax.experimental.pallas as pl
import jax.experimental.pallas.tpu as pltpu

S, D, H, DH, F = 2048, 640, 32, 20, 1728
HPG = 6
NG = 6
GW = NG * 128
QB = 512
NQB = S // QB
RC = 256
KC = 128
NKC = S // KC
UN = 8
EPS = 1e-5
QSCALE = (DH ** -0.5) * math.log2(math.e)

NT = (((1,), (1,)), ((), ()))


def _ln(x):
    m = jnp.mean(x, axis=-1, keepdims=True)
    xc = x - m
    v = jnp.mean(xc * xc, axis=-1, keepdims=True)
    return xc * jax.lax.rsqrt(v + EPS)


def _kernel(x_hbm, wqkv_ref, wo_hbm, w1_hbm, w3_hbm, w2_hbm, o_ref,
            wg_ref, wvT_ref, k2_ref, q2_ref, vtp_ref, ot_ref, sa_ref, sb_ref, ma_ref, mb_ref,
            wo_ref, w1_ref, w3_ref, w2_ref, x_ref, sems, xsems):
    step = pl.program_id(0)

    def late_copies():
        return [pltpu.make_async_copy(wo_hbm, wo_ref, sems.at[0]),
                pltpu.make_async_copy(w1_hbm, w1_ref, sems.at[1]),
                pltpu.make_async_copy(w3_hbm, w3_ref, sems.at[2]),
                pltpu.make_async_copy(w2_hbm, w2_ref, sems.at[3])]

    def x_copy(c):
        return pltpu.make_async_copy(x_hbm.at[pl.ds(c * RC, RC), :],
                                     x_ref.at[pl.ds(c * RC, RC), :], xsems.at[c])

    lane = jax.lax.broadcasted_iota(jnp.int32, (QB, 128), 1)

    def qweights(qbi, h):
        g = h // HPG
        j = h - g * HPG
        c0 = pl.multiple_of(g * 128, 128)
        lo = j * DH
        msk = (lane >= lo) & (lane < lo + DH)
        qq = q2_ref[pl.ds(pl.multiple_of(qbi * QB, QB), QB), pl.ds(c0, 128)]
        return jnp.where(msk, qq, jnp.zeros_like(qq)), c0

    def qk_chunk(qq, c0, sref, c, mx):
        kc = k2_ref[pl.ds(c * KC, KC), pl.ds(c0, 128)]
        s = jax.lax.dot_general(kc, qq, NT, preferred_element_type=jnp.float32)
        sref[pl.ds(c * KC, KC), :] = s
        sm = jnp.max(s.reshape(KC // 8, 8, QB), axis=0)
        return sm if mx is None else jnp.maximum(mx, sm)

    @pl.when(step == 0)
    def _phase1():
        for c in range(S // RC):
            x_copy(c).start()
        for cp in late_copies():
            cp.start()
        for g in range(NG):
            wg_ref[:, g * 128:(g + 1) * 128] = wqkv_ref[:, g * 120:g * 120 + 128]
            wg_ref[:, GW + g * 128:GW + (g + 1) * 128] = wqkv_ref[:, D + g * 120:D + g * 120 + 128]
        wvT_ref[...] = wqkv_ref[:, 2 * D:3 * D].astype(jnp.float32).T.astype(jnp.bfloat16)

        def chunk(c, carry):
            r0 = pl.multiple_of(c * RC, RC)
            x_copy(c).wait()
            x = x_ref[pl.ds(r0, RC), :].astype(jnp.float32)
            xl = _ln(x).astype(jnp.bfloat16)
            qk = jnp.dot(xl, wg_ref[...], preferred_element_type=jnp.float32)
            q2_ref[pl.ds(r0, RC), :] = (qk[:, :GW] * QSCALE).astype(jnp.bfloat16)
            k2_ref[pl.ds(r0, RC), :] = qk[:, GW:].astype(jnp.bfloat16)
            vt = jax.lax.dot_general(wvT_ref[...], xl, NT, preferred_element_type=jnp.float32)
            row = jax.lax.broadcasted_iota(jnp.int32, (32, RC), 0)
            for h in range(H):
                a = (DH * h // 8) * 8
                off = DH * h - a
                win = vt[a:a + 24, :]
                if off:
                    win = pltpu.roll(win, 24 - off, 0)
                win = jnp.concatenate([win, jnp.zeros((8, RC), jnp.float32)], axis=0)
                val = jnp.where(row < DH, win, jnp.where(row == DH, 1.0, 0.0))
                vtp_ref[h, :, pl.ds(r0, RC)] = val.astype(jnp.bfloat16)
            return carry
        jax.lax.fori_loop(0, S // RC, chunk, 0)

        qq, c0 = qweights(0, 0)
        mx = None
        for c in range(NKC):
            mx = qk_chunk(qq, c0, sa_ref, c, mx)
        ma_ref[...] = jnp.max(mx, axis=0, keepdims=True)

    @pl.when(step > 0)
    def _qblock():
        qb = step - 1
        q0 = pl.multiple_of(qb * QB, QB)

        def unit(h, qbn, hn, sc_ref, mc_ref, sn_ref, mn_ref):
            qq, c0 = qweights(qbn, hn)
            m = mc_ref[...]
            vt = vtp_ref[h]
            acc = jnp.zeros((32, QB), jnp.float32)
            mx = None
            for c in range(NKC):
                mx = qk_chunk(qq, c0, sn_ref, c, mx)
                sc = sc_ref[pl.ds(c * KC, KC), :]
                p = jnp.exp2(sc - m).astype(jnp.bfloat16)
                acc = acc + jnp.dot(vt[:, c * KC:(c + 1) * KC], p, preferred_element_type=jnp.float32)
            mn_ref[...] = jnp.max(mx, axis=0, keepdims=True)
            ot_ref[h, pl.ds(0, DH), :] = acc[:DH] / acc[DH:DH + 1]

        def group(i, carry):
            h0 = UN * i
            last = i == H // UN - 1
            for u in range(UN):
                h = h0 + u
                bufs = (sa_ref, ma_ref, sb_ref, mb_ref) if u % 2 == 0 else (sb_ref, mb_ref, sa_ref, ma_ref)
                if u < UN - 1:
                    unit(h, qb, h + 1, *bufs)
                else:
                    qbn = jnp.where(last, jnp.minimum(qb + 1, NQB - 1), qb)
                    hn = jnp.where(last, 0, h + 1)
                    unit(h, qbn, hn, *bufs)
            return carry
        jax.lax.fori_loop(0, H // UN, group, 0)

        @pl.when(step == 1)
        def _():
            for cp in late_copies():
                cp.wait()

        otf = jnp.concatenate([ot_ref[hh, 0:DH, :] for hh in range(H)], axis=0)
        attn = jnp.dot(otf.T.astype(jnp.bfloat16), wo_ref[...], preferred_element_type=jnp.float32)
        hres = x_ref[pl.ds(q0, QB), :].astype(jnp.float32) + attn
        l2 = _ln(hres).astype(jnp.bfloat16)
        gate = jax.lax.dot_general(l2, w1_ref[...], NT, preferred_element_type=jnp.float32)
        up = jax.lax.dot_general(l2, w3_ref[...], NT, preferred_element_type=jnp.float32)
        hf = (gate * jax.nn.sigmoid(gate) * up).astype(jnp.bfloat16)
        out = jnp.dot(hf, w2_ref[...], preferred_element_type=jnp.float32)
        o_ref[...] = (hres + out).astype(o_ref.dtype)


@jax.jit
def pallas_sequential_preLN__softmax_full_mha__glu_gated_swiglu__prompt_kernel(
    A_x: jax.Array,
    A_wqkv: jax.Array,
    A_wo: jax.Array,
    B_x: jax.Array,
    B_w1: jax.Array,
    B_w3: jax.Array,
    B_w2: jax.Array,
):
    x = A_x.reshape(S, D)
    anyspec = pl.BlockSpec(memory_space=pl.ANY)
    out = pl.pallas_call(
        _kernel,
        grid=(1 + NQB,),
        in_specs=[anyspec, pl.BlockSpec((D, 3 * D), lambda i: (0, 0)), anyspec, anyspec, anyspec, anyspec],
        out_specs=pl.BlockSpec((QB, D), lambda i: (jnp.maximum(i - 1, 0), 0)),
        out_shape=jax.ShapeDtypeStruct((S, D), jnp.bfloat16),
        scratch_shapes=[
            pltpu.VMEM((D, 2 * GW), jnp.bfloat16),
            pltpu.VMEM((D, D), jnp.bfloat16),
            pltpu.VMEM((S, GW), jnp.bfloat16),
            pltpu.VMEM((S, GW), jnp.bfloat16),
            pltpu.VMEM((H, 32, S), jnp.bfloat16),
            pltpu.VMEM((H, 24, QB), jnp.float32),
            pltpu.VMEM((S, QB), jnp.float32),
            pltpu.VMEM((S, QB), jnp.float32),
            pltpu.VMEM((1, QB), jnp.float32),
            pltpu.VMEM((1, QB), jnp.float32),
            pltpu.VMEM((D, D), jnp.bfloat16),
            pltpu.VMEM((F, D), jnp.bfloat16),
            pltpu.VMEM((F, D), jnp.bfloat16),
            pltpu.VMEM((F, D), jnp.bfloat16),
            pltpu.VMEM((S, D), jnp.bfloat16),
            pltpu.SemaphoreType.DMA((4,)),
            pltpu.SemaphoreType.DMA((S // RC,)),
        ],
        compiler_params=pltpu.CompilerParams(dimension_semantics=("arbitrary",),
                                             vmem_limit_bytes=100 * 1024 * 1024),
    )(x, A_wqkv, A_wo, B_w1.T, B_w3.T, B_w2)
    return out.reshape(1, S, D)
```
